```python
import os as _os
_os.environ.setdefault("JAX_PLATFORMS", "cpu")
import jax
import jax.numpy as jnp

def _softmax(x, axis=-1):
    return jax.nn.softmax(x, axis=axis)
def _gelu(x):
    return jax.nn.gelu(x, approximate=True)
def _silu(x):
    return jax.nn.silu(x)
def _sigmoid(x):
    return jax.nn.sigmoid(x)
def _layernorm(x, axis=-1, eps=1e-5):
    m = jnp.mean(x, axis=axis, keepdims=True)
    v = jnp.var(x, axis=axis, keepdims=True)
    return (x - m) / jnp.sqrt(v + eps)
def _scatter_add(tgt, idx, src, axis=0):
    return tgt.at[idx].add(src)
def _segment_sum(src, seg, n):
    return jax.ops.segment_sum(src, seg, n)
class _Rng:
    def __init__(self, key):
        self._k = key
    def _next(self):
        self._k, sub = jax.random.split(self._k)
        return sub
    def normal(self, shape):
        return jax.random.normal(self._next(), shape, dtype=jnp.bfloat16)
    def randint(self, lo, hi, shape):
        return jax.random.randint(self._next(), shape, lo, hi, dtype=jnp.int32)
    def uniform(self, shape, lo=0.0, hi=1.0):
        return jax.random.uniform(self._next(), shape, jnp.bfloat16, lo, hi)
    def permutation(self, n):
        return jax.random.permutation(self._next(), n)


kernel_name = 'standalone__mha_block_cached__near_ridge'

def setup_inputs():
    _rng = _Rng(jax.random.key(int.from_bytes(__import__("os").urandom(4), "little")))
    _w = (lambda a: (lambda t: t.astype(jnp.bfloat16) if jnp.issubdtype(t.dtype, jnp.floating) else t)(jnp.asarray(a)))
    B, Sq, D = 8, 96, 576
    H, Sk, Dh = 32, 96, 128
    return {
        "x": _w((lambda *s: _rng.normal(s) * 0.8)(B, Sq, D)),
        "k_cache": _w((lambda *s: _rng.normal(s) * 0.8)(B, H, Sk, Dh)),
        "v_cache": _w((lambda *s: _rng.normal(s) * 0.05)(B, H, Sk, Dh)),
        "wq": _w((lambda *s: _rng.normal(s) * 0.8)(D, H * Dh) * (D ** -0.5)),
        "wo": _w((lambda *s: _rng.normal(s) * 0.05)(H * Dh, D) * ((H * Dh) ** -0.5)),
    }

def reference(x, k_cache, v_cache, wq, wo):
    B, Sq, D = x.shape
    H, Dh = 32, 128
    q = (lambda x, *d: x.transpose(*d))((x @ wq).reshape(B, Sq, H, Dh), 0, 2, 1, 3)
    scores = jnp.einsum("bhqd,bhkd->bhqk", q, k_cache) * (Dh ** -0.5)
    p = _softmax(scores, axis=-1)
    o = jnp.einsum("bhqk,bhkd->bhqd", p, v_cache)
    return (lambda x, *d: x.transpose(*d))(o, 0, 2, 1, 3).reshape(B, Sq, H * Dh) @ wo
```

```python
import functools, contextlib
import jax
import jax.numpy as jnp
from jax import lax
import jax.experimental.pallas as pl
import jax.experimental.pallas.tpu as pltpu

B, SQ, D = 8, 96, 576
H, SK, DH = 32, 96, 128
M = B * SQ
NT = (((1,), (1,)), ((), ()))
C = (DH ** -0.5) * 1.4426950408889634
G = 4; NG = H // G; W = G * DH; NP = H // 2
HD, HM, HW = D // 2, M // 2, W // 2
TR = 128
f32, bf = jnp.float32, jnp.bfloat16
RND = []
for _i in (0, 2, 4):
    RND += [[(_i, 0, 256)], [(_i, 256, 128), (_i+1, 0, 128)], [(_i+1, 128, 256)]]
RND += [[(6, 0, 256)], [(6, 256, 128)]]
ORD = "q0 r0 q1 q2 r1 p0 r3 q3 p1 r2 p2 r4 q5 q4 r5 q6 p3 r6 p4 r7 q7 p5 r8 p6 p7 r9 r10"
ORD0 = "q0 q1 f0 q2 p0 q3 p1 f1 q4 p2 q5 p3 f2 q6 p4 q7 p5 f3 p6 p7"

def make(per=3, order=ORD, order0=ORD0, order7=None, scopes=False, only=None, chain=True, ga=3, link=1, px=4, pa=8, nb=False):
    order = order.split(); order0 = order0.split(); order7 = order7.split() if order7 else order
    sc = (lambda n: jax.named_scope(n)) if scopes else (lambda n: contextlib.nullcontext())
    def body(x_hbm, k_hbm, v_hbm, wq_hbm, wot_hbm, o_hbm,
             x_v, k_v, v_v, wq_v, wot_v, q_v, o0, o1, xs, acc, out_v, sem, sm):
        os_ = (o0, o1)
        def mo(i, n): return i * n if isinstance(i, int) else pl.multiple_of(i * n, n)
        def cx(i): return pltpu.make_async_copy(x_hbm.at[pl.ds(mo(i, HM), HM)], x_v.at[pl.ds(mo(i, HM), HM)], sem.at[i])
        def cq(i, s_): return pltpu.make_async_copy(wq_hbm.at[:, pl.ds(mo(i, 2*DH), 2*DH)], wq_v.at[i, 0:D], sem.at[s_])
        def co(g, s_): return pltpu.make_async_copy(wot_hbm.at[:, pl.ds(mo(g, W), W)], wot_v.at[g, 0:D], sem.at[s_])
        def ck(g): return pltpu.make_async_copy(k_hbm.at[:, pl.ds(g*G, G)], k_v.at[g], sem.at[7 + (g + 1) // 2])
        def cv(g): return pltpu.make_async_copy(v_hbm.at[:, pl.ds(g*G, G)], v_v.at[g], sem.at[7 + (g + 1) // 2])
        def cout(j): return pltpu.make_async_copy(out_v.at[pl.ds(mo(j, TR), TR)], o_hbm.at[pl.ds(mo(j, TR), TR)], sem.at[0])

        def qproj(i, r0=0, nr=M):
            q = jnp.dot(x_v[r0:r0+nr, :], wq_v[i, 0:D], preferred_element_type=f32)
            q_v[i, r0:r0+nr, :] = q.astype(bf)
        def xsums():
            z = 0
            for r0 in range(0, HM, 16):
                for _ in range(px): z = sm[z]
                lo, hi = pl.ds(pl.multiple_of(z + r0, 16), 16), pl.ds(pl.multiple_of(z + HM + r0, 16), 16)
                a11 = x_v[lo, 0:256].astype(f32); a12 = x_v[lo, 256:512].astype(f32)
                a21 = x_v[hi, 0:256].astype(f32); a22 = x_v[hi, 256:512].astype(f32)
                for i, a in enumerate([a11 + a22, a21 + a22, a11 + a12, a21 - a11, a12 - a22]):
                    xs[i, r0:r0+16, :] = a.astype(bf)
        def wsums(i, part, nparts):
            n = 256 // nparts
            for r0 in range(part * n, (part + 1) * n, 16):
                lo = wq_v[i, r0:r0+16, :].astype(f32); hi = wq_v[i, 256+r0:256+r0+16, :].astype(f32)
                b11, b12, b21, b22 = lo[:, :DH], lo[:, DH:], hi[:, :DH], hi[:, DH:]
                for j, a in enumerate([b11 + b22, b12 - b22, b21 - b11, b11 + b12, b21 + b22]):
                    wq_v[i, D + j*256 + r0: D + j*256 + r0 + 16, 0:DH] = a.astype(bf)
        def qproj_s(i, nxt, own=False):
            if own: wsums(i, 0, 1)
            rl = jnp.dot(x_v[0:HM, 512:D], wq_v[i, 512:D, :], preferred_element_type=f32)
            rh = jnp.dot(x_v[HM:M, 512:D], wq_v[i, 512:D, :], preferred_element_type=f32)
            ws_ = lambda j: wq_v[i, D + j*256: D + (j+1)*256, 0:DH]
            A = [lambda: xs[0], lambda: xs[1], lambda: x_v[0:HM, 0:256], lambda: x_v[HM:M, 256:512], lambda: xs[2], lambda: xs[3], lambda: xs[4]]
            Bm = [lambda: ws_(0), lambda: wq_v[i, 0:256, 0:DH], lambda: ws_(1), lambda: ws_(2), lambda: wq_v[i, 256:512, DH:2*DH], lambda: ws_(3), lambda: ws_(4)]
            m = [None] * 7
            for n, j in enumerate((1, 4, 3, 2, 0, 6, 5)):
                m[j] = jnp.dot(A[j](), Bm[j](), preferred_element_type=f32)
                if n % 2 == 1 and nxt is not None: wsums(nxt, n // 2, 4)
            if nxt is not None: wsums(nxt, 3, 4)
            q_v[i, 0:HM, 0:DH] = (rl[:, :DH] - m[4] + m[3] + m[0] + m[6]).astype(bf)
            q_v[i, 0:HM, DH:] = (rl[:, DH:] + m[4] + m[2]).astype(bf)
            q_v[i, HM:M, 0:DH] = (rh[:, :DH] + m[1] + m[3]).astype(bf)
            q_v[i, HM:M, DH:] = (rh[:, DH:] - m[1] + m[2] + m[0] + m[5]).astype(bf)
        zz = [0]
        def asum(g, z16):
            L = 16 * link
            g0 = g
            for r0 in range(0, HD, L):
                for _ in range(pa): zz[0] = sm[zz[0]]
                g = g0 + zz[0]
                a11 = wot_v[g, r0:r0+L, 0:HW]; a12 = wot_v[g, r0:r0+L, HW:W]
                a21 = wot_v[g, HD+r0:HD+r0+L, 0:HW]; a22 = wot_v[g, HD+r0:HD+r0+L, HW:W]
                a11, a12, a21, a22 = [a.astype(f32) for a in (a11, a12, a21, a22)]
                for i, a in enumerate([a11 + a22, a21 + a22, a11 + a12, a21 - a11, a12 - a22]):
                    wot_v[g, pl.ds(pl.multiple_of(z16 + D + i*HD + r0, 16), L), 0:HW] = a.astype(bf)
        def qk1(g, b, h):
            r0 = min(b*SQ, M - 128)
            qb = q_v[2*g + h//2, r0:r0+128, (h%2)*DH:(h%2+1)*DH]
            s = lax.dot_general(k_v[g, b, h], qb, NT, preferred_element_type=f32)
            m = jnp.max(s, axis=0, keepdims=True)
            e = jnp.exp2((s - m) * C)
            l = jnp.sum(e, axis=0, keepdims=True)
            p = (e * (1.0 / l)).astype(bf).T
            return p[b*SQ - r0: b*SQ - r0 + SQ]
        def quad(n):
            b, h = n // 2, n % 2
            return [(b, h), (b+4, h), (b, h+2), (b+4, h+2)]
        def pv(g, par, n, ps):
            b11, b12, b21, b22 = [jnp.dot(p, v_v[g, b, h], preferred_element_type=f32) for p, (b, h) in zip(ps, quad(n))]
            b, h = quad(n)[0]
            for i, o in enumerate([b11 + b22, b11, b12 - b22, b21 - b11, b22, b11 + b12, b21 + b22]):
                os_[par][i, b*SQ:(b+1)*SQ, h*DH:(h+1)*DH] = o.astype(bf)
        def oprod(g, par, i, c0, nc, r0=0, r1=HD):
            if i == 2: a = wot_v[g, r0:r1, 0:HW]
            elif i == 3: a = wot_v[g, HD+r0:HD+r1, HW:W]
            else:
                j = {0:0, 1:1, 4:2, 5:3, 6:4}[i]
                a = wot_v[g, D + j*HD + r0: D + j*HD + r1, 0:HW]
            return lax.dot_general(a, os_[par][i, c0:c0+nc, :], NT, preferred_element_type=f32)
        def stage(g, par, order):
            ps = {}
            for it in order:
                n = int(it[1:])
                if it[0] == "q": ps[n] = [qk1(g, b, h) for b, h in quad(n)]
                if it[0] == "p": pv(g, par, n, ps.pop(n))
                if it[0] == "r":
                    for i, c0, nc in RND[n]: acc[i, :, c0:c0+nc] += oprod(g-1, 1-par, i, c0, nc)
                if it[0] == "f": qproj(NP - 2 + n // 2, (n % 2) * HM, HM)
        def final(j):
            m = [None] * 7
            for i in (0, 1, 3, 4, 6, 2): m[i] = acc[i, :, j*TR:(j+1)*TR] + oprod(7, 1, i, j*TR, TR)
            m5 = jnp.concatenate([oprod(7, 1, 5, j*TR, TR, 0, HD//2), oprod(7, 1, 5, j*TR, TR, HD//2, HD)], axis=0)
            c11 = m[0] + m[3] - m[4] + m[6]; c12 = m[2] + m[4]; c21 = m[1] + m[3]; c22 = m[0] - m[1] + m[2] + acc[5, :, j*TR:(j+1)*TR] + m5
            out_v[j*TR:(j+1)*TR, :] = jnp.concatenate([c11, c21], axis=0).T.astype(bf)
            out_v[HM+j*TR:HM+(j+1)*TR, :] = jnp.concatenate([c12, c22], axis=0).T.astype(bf)
        def lp2(i, c):
            g = 1 + 2*i
            with sc("rB"):
                if only is None:
                    for gg in (g, g+1): ck(gg).wait(); cv(gg).wait()
                stage(g, 1, order)
                stage(g+1, 0, order)
            return c
        if only == "B":
            lax.fori_loop(0, 3, lp2, 0); return

        nA = 3
        cx(0).start(); cq(0, 0).start()
        def i0(i, c):
            @pl.when(i == 0)
            def _(): cx(1).start()
            @pl.when(i > 0)
            def _(): cq(i, 2 + i // 3).start()
            @pl.when(jnp.logical_and(i >= 6, i < 6 + NG))
            def _(): co(i - 6, 2 + i // 3).start()
            return c
        lax.fori_loop(0, NP, i0, 0)
        def i2(g, c):
            ck(g).start(); cv(g).start(); return c
        lax.fori_loop(0, NG, i2, 0)
        sm[0] = 0
        with sc("w0"): cx(0).wait(); cq(0, 0).wait()
        with sc("r0"): qproj(0, 0, HM // 2); qproj(0, HM // 2, HM // 2)
        with sc("w1"): cx(1).wait()
        with sc("r1"):
            qproj(0, HM, HM // 2); xsums(); qproj(0, HM + HM // 2, HM // 2)
        with sc("w2"):
            for u in (1, 2): cq(u, 2).wait()
        with sc("r2a"):
            qproj_s(1, 2, True); qproj_s(2, None)
        with sc("w3"):
            for u in (3, 4, 5): cq(u, 3).wait()
        with sc("r2b"):
            qproj_s(3, 4, True); acc[...] = jnp.zeros_like(acc); qproj_s(4, 5)
        def lq(i, c):
            with sc("rA"):
                for u in range(3):
                    cq(6 + i*3 + u, 4 + i).wait()
                    if u < 2: co(i*3 + u, 4 + i).wait()
                    else:
                        @pl.when(i < 2)
                        def _(): co(i*3 + u, 4 + i).wait()
                z16 = sm[0] * 16; zz[0] = 0
                for u in range(3):
                    qproj_s(5 + i*3 + u, 6 + i*3 + u)
                    asum(jnp.minimum(i*3 + u, NG - 1), z16)
            return c
        lax.fori_loop(0, nA, lq, 0)
        with sc("s0"):
            cq(15, 7).wait(); ck(0).wait(); cv(0).wait()
            stage(0, 0, order0)
        lax.fori_loop(0, 3, lp2, 0)
        with sc("s7"):
            ck(7).wait(); cv(7).wait()
            stage(7, 1, order7)
            final(0); final(1)
        def st(i, c):
            cout(i).start(); cout(i + 3).start(); return c
        lax.fori_loop(0, 2, st, 0)
        with sc("f2"): final(2)
        with sc("end"):
            cout(2).start(); cout(5).start()
            for j in range(6): cout(j).wait()

    @jax.jit
    def fn(x, k_cache, v_cache, wq, wo):
        anyspec = pl.BlockSpec(memory_space=pltpu.HBM)
        out = pl.pallas_call(
            body,
            in_specs=[anyspec]*5, out_specs=anyspec,
            out_shape=jax.ShapeDtypeStruct((M, D), bf),
            scratch_shapes=[pltpu.VMEM((M, D), bf), pltpu.VMEM((NG, B, G, SK, DH), bf), pltpu.VMEM((NG, B, G, SK, DH), bf),
                            pltpu.VMEM((NP, D + 5*256, 2*DH), bf), pltpu.VMEM((NG, D + 5*HD, W), bf),
                            pltpu.VMEM((NP, M, 2*DH), bf), pltpu.VMEM((7, HM, HW), bf), pltpu.VMEM((7, HM, HW), bf),
                            pltpu.VMEM((5, HM, 256), bf),
                            pltpu.VMEM((7, HD, HM), f32), pltpu.VMEM((M, D), bf),
                            pltpu.SemaphoreType.DMA((12,)), pltpu.SMEM((1,), jnp.int32)],
            compiler_params=pltpu.CompilerParams(vmem_limit_bytes=100*1024*1024, disable_bounds_checks=nb),
        )(x.reshape(M, D), k_cache, v_cache, wq, wo.T)
        return out.reshape(B, SQ, D)
    return fn

pallas_standalone__mha_block_cached__near_ridge_kernel = make()
```

```python
import jax
import jax.numpy as jnp
from jax import lax
import jax.experimental.pallas as pl
import jax.experimental.pallas.tpu as pltpu

B, SQ, D = 8, 96, 576
H, SK, DH = 32, 96, 128
M = B * SQ
G = 4
NG = H // G
W = G * DH
NP = H // 2
HD, HM, HW = D // 2, M // 2, W // 2
KS = 256
TR = 128
NT = (((1,), (1,)), ((), ()))
EXP2_SCALE = (DH ** -0.5) * 1.4426950408889634
f32, bf16 = jnp.float32, jnp.bfloat16

ROUNDS = []
for _i in (0, 2, 4):
    ROUNDS += [[(_i, 0, 256)], [(_i, 256, 128), (_i + 1, 0, 128)], [(_i + 1, 128, 256)]]
ROUNDS += [[(6, 0, 256)], [(6, 256, 128)]]

ORDER_FIRST = "q0 q1 s0 q2 p0 p1 q4 p2 q3 s1 q5 q6 q7 p3 p4 p5 p6 p7".split()
ORDER_MAIN = ("q0 r0 q1 q2 r1 p0 r3 q3 p1 r2 p2 r4 q5 q4 r5 q6 p3 r6 p4 r7 q7 p5 r8 p6 p7 "
              "r9 r10").split()
ORDER_LAST = ("q0 q1 r0 q2 r3 r1 p0 p1 q3 r2 p2 q5 r5 q4 q6 r4 p3 p4 r8 q7 r7 r6 p5 r10 p7 "
              "r9 p6").split()
PACE_X, PACE_W = 4, 6


def _lhs_sums(a11, a12, a21, a22):
    a11, a12, a21, a22 = (a.astype(f32) for a in (a11, a12, a21, a22))
    return [a11 + a22, a21 + a22, a11 + a12, a21 - a11, a12 - a22]


def _kernel(x_hbm, k_hbm, v_hbm, wq_hbm, wot_hbm, o_hbm,
            x_v, k_v, v_v, wq_v, wot_v, q_v, o0, o1, xs, acc, out_v, sem, zero):
    o_bufs = (o0, o1)

    def mo(i, n):
        return i * n if isinstance(i, int) else pl.multiple_of(i * n, n)

    def cx(i):
        return pltpu.make_async_copy(
            x_hbm.at[pl.ds(mo(i, HM), HM)], x_v.at[pl.ds(mo(i, HM), HM)], sem.at[i])

    def cq(i, s):
        return pltpu.make_async_copy(
            wq_hbm.at[:, pl.ds(mo(i, 2 * DH), 2 * DH)], wq_v.at[i, 0:D], sem.at[s])

    def co(g, s):
        return pltpu.make_async_copy(
            wot_hbm.at[:, pl.ds(mo(g, W), W)], wot_v.at[g, 0:D], sem.at[s])

    def ck(g):
        return pltpu.make_async_copy(
            k_hbm.at[:, pl.ds(g * G, G)], k_v.at[g], sem.at[7 + (g + 1) // 2])

    def cv(g):
        return pltpu.make_async_copy(
            v_hbm.at[:, pl.ds(g * G, G)], v_v.at[g], sem.at[7 + (g + 1) // 2])

    def cout(j):
        return pltpu.make_async_copy(
            out_v.at[pl.ds(mo(j, TR), TR)], o_hbm.at[pl.ds(mo(j, TR), TR)], sem.at[0])

    def kv_start(g):
        ck(g).start()
        cv(g).start()

    def pace(z, n):
        for _ in range(n):
            z = zero[z]
        return z

    def qproj(i, r0, nr):
        q = jnp.dot(x_v[r0:r0 + nr, :], wq_v[i, 0:D], preferred_element_type=f32)
        q_v[i, r0:r0 + nr, :] = q.astype(bf16)

    def x_sums():
        z = 0
        for r0 in range(0, HM, 16):
            z = pace(z, PACE_X)
            lo = pl.ds(pl.multiple_of(z + r0, 16), 16)
            hi = pl.ds(pl.multiple_of(z + HM + r0, 16), 16)
            sums = _lhs_sums(x_v[lo, 0:KS], x_v[lo, KS:2 * KS], x_v[hi, 0:KS], x_v[hi, KS:2 * KS])
            for i, a in enumerate(sums):
                xs[i, r0:r0 + 16, :] = a.astype(bf16)

    def wq_sums(i, part, nparts):
        n = KS // nparts
        for r0 in range(part * n, (part + 1) * n, 16):
            lo = wq_v[i, r0:r0 + 16, :].astype(f32)
            hi = wq_v[i, KS + r0:KS + r0 + 16, :].astype(f32)
            b11, b12, b21, b22 = lo[:, :DH], lo[:, DH:], hi[:, :DH], hi[:, DH:]
            for j, b in enumerate([b11 + b22, b12 - b22, b21 - b11, b11 + b12, b21 + b22]):
                wq_v[i, D + j * KS + r0:D + j * KS + r0 + 16, 0:DH] = b.astype(bf16)

    def qproj_strassen(i, nxt, own_sums=False):
        if own_sums:
            wq_sums(i, 0, 1)
        rl = jnp.dot(x_v[0:HM, 2 * KS:D], wq_v[i, 2 * KS:D, :], preferred_element_type=f32)
        rh = jnp.dot(x_v[HM:M, 2 * KS:D], wq_v[i, 2 * KS:D, :], preferred_element_type=f32)

        def ws(j):
            return wq_v[i, D + j * KS:D + (j + 1) * KS, 0:DH]

        lhs = [lambda: xs[0], lambda: xs[1], lambda: x_v[0:HM, 0:KS],
               lambda: x_v[HM:M, KS:2 * KS], lambda: xs[2], lambda: xs[3], lambda: xs[4]]
        rhs = [lambda: ws(0), lambda: wq_v[i, 0:KS, 0:DH], lambda: ws(1), lambda: ws(2),
               lambda: wq_v[i, KS:2 * KS, DH:2 * DH], lambda: ws(3), lambda: ws(4)]
        m = [None] * 7
        for n, j in enumerate((1, 4, 3, 2, 0, 6, 5)):
            m[j] = jnp.dot(lhs[j](), rhs[j](), preferred_element_type=f32)
            if n % 2 == 1 and nxt is not None:
                wq_sums(nxt, n // 2, 4)
        if nxt is not None:
            wq_sums(nxt, 3, 4)
        q_v[i, 0:HM, 0:DH] = (rl[:, :DH] - m[4] + m[3] + m[0] + m[6]).astype(bf16)
        q_v[i, 0:HM, DH:] = (rl[:, DH:] + m[4] + m[2]).astype(bf16)
        q_v[i, HM:M, 0:DH] = (rh[:, :DH] + m[1] + m[3]).astype(bf16)
        q_v[i, HM:M, DH:] = (rh[:, DH:] - m[1] + m[2] + m[0] + m[5]).astype(bf16)

    def quad(n):
        b, h = n // 2, n % 2
        return [(b, h), (b + B // 2, h), (b, h + 2), (b + B // 2, h + 2)]

    def probs(g, b, h):
        r0 = min(b * SQ, M - 128)
        q = q_v[2 * g + h // 2, r0:r0 + 128, (h % 2) * DH:(h % 2 + 1) * DH]
        s = lax.dot_general(k_v[g, b, h], q, NT, preferred_element_type=f32)
        m = jnp.max(s, axis=0, keepdims=True)
        e = jnp.exp2((s - m) * EXP2_SCALE)
        l = jnp.sum(e, axis=0, keepdims=True)
        p = (e * (1.0 / l)).astype(bf16).T
        return p[b * SQ - r0:b * SQ - r0 + SQ]

    def pv(g, par, n, ps):
        b11, b12, b21, b22 = [jnp.dot(p, v_v[g, b, h], preferred_element_type=f32)
                              for p, (b, h) in zip(ps, quad(n))]
        b, h = quad(n)[0]
        for i, o in enumerate([b11 + b22, b11, b12 - b22, b21 - b11, b22, b11 + b12, b21 + b22]):
            o_bufs[par][i, b * SQ:(b + 1) * SQ, h * DH:(h + 1) * DH] = o.astype(bf16)

    def wo_sums(g, z, z16):
        for r0 in range(0, HD, 16):
            z = pace(z, PACE_W)
            gz = g + z
            sums = _lhs_sums(wot_v[gz, r0:r0 + 16, 0:HW], wot_v[gz, r0:r0 + 16, HW:W],
                             wot_v[gz, HD + r0:HD + r0 + 16, 0:HW],
                             wot_v[gz, HD + r0:HD + r0 + 16, HW:W])
            for i, a in enumerate(sums):
                rows = pl.ds(pl.multiple_of(z16 + D + i * HD + r0, 16), 16)
                wot_v[gz, rows, 0:HW] = a.astype(bf16)
        return z

    def oprod(g, par, i, c0, nc, r0=0, r1=HD):
        if i == 2:
            a = wot_v[g, r0:r1, 0:HW]
        elif i == 3:
            a = wot_v[g, HD + r0:HD + r1, HW:W]
        else:
            j = {0: 0, 1: 1, 4: 2, 5: 3, 6: 4}[i]
            a = wot_v[g, D + j * HD + r0:D + j * HD + r1, 0:HW]
        return lax.dot_general(a, o_bufs[par][i, c0:c0 + nc, :], NT, preferred_element_type=f32)

    def stage(g, par, order):
        ps = {}
        for item in order:
            kind, n = item[0], int(item[1:])
            if kind == "q":
                ps[n] = [probs(g, b, h) for b, h in quad(n)]
            elif kind == "p":
                pv(g, par, n, ps.pop(n))
            elif kind == "r":
                for i, c0, nc in ROUNDS[n]:
                    acc[i, :, c0:c0 + nc] += oprod(g - 1, 1 - par, i, c0, nc)
            else:
                qproj_strassen(NP - 2 + n, NP - 1 if n == 0 else None)

    def last_head_start(j):
        cols = slice(j * TR, (j + 1) * TR)
        for i in (0, 1, 3, 4):
            acc[i, :, cols] += oprod(NG - 1, 1, i, j * TR, TR)

    def last_finish(j, done):
        cols = slice(j * TR, (j + 1) * TR)
        m = [None] * 7
        for t, i in enumerate((0, 1, 3, 4, 6, 2)):
            m[i] = acc[i, :, cols]
            if t >= done:
                m[i] = m[i] + oprod(NG - 1, 1, i, j * TR, TR)
        m5 = jnp.concatenate([oprod(NG - 1, 1, 5, j * TR, TR, 0, HD // 2),
                              oprod(NG - 1, 1, 5, j * TR, TR, HD // 2, HD)], axis=0)
        c11 = m[0] + m[3] - m[4] + m[6]
        c12 = m[2] + m[4]
        c21 = m[1] + m[3]
        c22 = m[0] - m[1] + m[2] + acc[5, :, cols] + m5
        out_v[j * TR:(j + 1) * TR, :] = jnp.concatenate([c11, c21], axis=0).T.astype(bf16)
        out_v[HM + j * TR:HM + (j + 1) * TR, :] = jnp.concatenate([c12, c22], axis=0).T.astype(bf16)

    def out_start(j):
        def body(i, c):
            cout(j + 3 * i).start()
            return c
        lax.fori_loop(0, 2, body, 0)

    cx(0).start()
    cq(0, 0).start()

    def issue(i, c):
        @pl.when(i == 0)
        def _():
            cx(1).start()

        @pl.when(i > 0)
        def _():
            cq(i, 2 + i // 3).start()

        @pl.when(jnp.logical_and(i >= 6, i < 6 + NG))
        def _():
            co(i - 6, 2 + i // 3).start()
        return c

    lax.fori_loop(0, NP, issue, 0)
    zero[0] = 0
    acc[...] = jnp.zeros_like(acc)

    cx(0).wait()
    cq(0, 0).wait()
    qproj(0, 0, HM // 2)
    qproj(0, HM // 2, HM // 2)

    cx(1).wait()
    qproj(0, HM, HM // 2)
    x_sums()
    qproj(0, HM + HM // 2, HM // 2)

    for u in (1, 2):
        cq(u, 2).wait()
    kv_start(0)
    qproj_strassen(1, 2, own_sums=True)
    qproj_strassen(2, None)

    for u in (3, 4, 5):
        cq(u, 3).wait()
    kv_start(1)
    kv_start(2)
    qproj_strassen(3, 4, own_sums=True)
    qproj_strassen(4, 5)

    def phase_a(i, c):
        for u in range(3):
            cq(6 + 3 * i + u, 4 + i).wait()
            if u < 2:
                co(3 * i + u, 4 + i).wait()
            else:
                @pl.when(i < 2)
                def _():
                    co(3 * i + u, 4 + i).wait()
        kv_start(3 + i)
        z16 = zero[0] * 16
        z = 0
        for u in range(3):
            qproj_strassen(5 + 3 * i + u, 6 + 3 * i + u)
            z = wo_sums(jnp.minimum(3 * i + u, NG - 1), z, z16)
        return c

    lax.fori_loop(0, 3, phase_a, 0)

    cq(NP - 1, 7).wait()
    ck(0).wait()
    cv(0).wait()
    kv_start(6)
    kv_start(7)
    stage(0, 0, ORDER_FIRST)

    def phase_b(i, c):
        g = 1 + 2 * i
        for gg in (g, g + 1):
            ck(gg).wait()
            cv(gg).wait()
        stage(g, 1, ORDER_MAIN)
        stage(g + 1, 0, ORDER_MAIN)
        return c

    lax.fori_loop(0, 3, phase_b, 0)

    ck(NG - 1).wait()
    cv(NG - 1).wait()
    stage(NG - 1, 1, ORDER_LAST)
    last_finish(0, 0)
    last_head_start(1)
    out_start(0)
    last_finish(1, 4)
    last_head_start(2)
    out_start(1)
    last_finish(2, 4)
    cout(2).start()
    cout(5).start()
    for j in range(6):
        cout(j).wait()


@jax.jit
def pallas_standalone__mha_block_cached__near_ridge_kernel(
    x: jax.Array,
    k_cache: jax.Array,
    v_cache: jax.Array,
    wq: jax.Array,
    wo: jax.Array,
):
    hbm = pl.BlockSpec(memory_space=pltpu.HBM)
    out = pl.pallas_call(
        _kernel,
        in_specs=[hbm] * 5,
        out_specs=hbm,
        out_shape=jax.ShapeDtypeStruct((M, D), bf16),
        scratch_shapes=[
            pltpu.VMEM((M, D), bf16),
            pltpu.VMEM((NG, B, G, SK, DH), bf16),
            pltpu.VMEM((NG, B, G, SK, DH), bf16),
            pltpu.VMEM((NP, D + 5 * KS, 2 * DH), bf16),
            pltpu.VMEM((NG, D + 5 * HD, W), bf16),
            pltpu.VMEM((NP, M, 2 * DH), bf16),
            pltpu.VMEM((7, HM, HW), bf16),
            pltpu.VMEM((7, HM, HW), bf16),
            pltpu.VMEM((5, HM, KS), bf16),
            pltpu.VMEM((7, HD, HM), f32),
            pltpu.VMEM((M, D), bf16),
            pltpu.SemaphoreType.DMA((12,)),
            pltpu.SMEM((1,), jnp.int32),
        ],
        compiler_params=pltpu.CompilerParams(vmem_limit_bytes=100 * 1024 * 1024),
    )(x.reshape(M, D), k_cache, v_cache, wq, wo.T)
    return out.reshape(B, SQ, D)
```
